```python
import os as _os
_os.environ.setdefault('JAX_PLATFORMS', 'cpu')
import jax
import jax.numpy as jnp

def _softmax(x, axis=-1):
    return jax.nn.softmax(x, axis=axis)

def _gelu(x):
    return jax.nn.gelu(x, approximate=True)

def _silu(x):
    return jax.nn.silu(x)

def _sigmoid(x):
    return jax.nn.sigmoid(x)

def _layernorm(x, axis=-1, eps=1e-05):
    m = jnp.mean(x, axis=axis, keepdims=True)
    v = jnp.var(x, axis=axis, keepdims=True)
    return (x - m) / jnp.sqrt(v + eps)

def _scatter_add(tgt, idx, src, axis=0):
    return tgt.at[idx].add(src)

def _segment_sum(src, seg, n):
    return jax.ops.segment_sum(src, seg, n)

class _Rng:

    def __init__(self, key):
        self._k = key

    def _next(self):
        self._k, sub = jax.random.split(self._k)
        return sub

    def normal(self, shape):
        return jax.random.normal(self._next(), shape, dtype=jnp.bfloat16)

    def randint(self, lo, hi, shape):
        return jax.random.randint(self._next(), shape, lo, hi, dtype=jnp.int32)

    def uniform(self, shape, lo=0.0, hi=1.0):
        return jax.random.uniform(self._next(), shape, jnp.bfloat16, lo, hi)

    def permutation(self, n):
        return jax.random.permutation(self._next(), n)
kernel_name = 'parallel_sum__memory_aug_recurrent_mem_tr__dense_activation_gelu__prompt'

def setup_inputs():
    _rng = _Rng(jax.random.key(int.from_bytes(__import__("os").urandom(4), "little")))
    _w = lambda a: (lambda t: t.astype(jnp.bfloat16) if jnp.issubdtype(t.dtype, jnp.floating) else t)(jnp.asarray(a))

    def _A_setup():
        B, S, Dm = (1, 2048, 1024)
        H, Dh = (32, 128)
        M, seg = (8, 32)
        seg = min(seg, S)
        S = S // seg * seg
        return {'x': _w((lambda *s: _rng.normal(s) * 0.05)(B, S, Dm)), 'mem0': _w((lambda *s: _rng.normal(s) * 0.2)(B, M, Dm)), 'Wq': _w((lambda *s: _rng.normal(s) * 0.8)(Dm, H, Dh) * Dm ** (-0.5)), 'Wk': _w((lambda *s: _rng.normal(s) * 0.8)(Dm, H, Dh) * Dm ** (-0.5)), 'Wv': _w((lambda *s: _rng.normal(s) * 0.2)(Dm, H, Dh) * Dm ** (-0.5)), 'Wo': _w((lambda *s: _rng.normal(s) * 0.2)(H, Dh, Dm) * (H * Dh) ** (-0.5)), 'seg_len': seg}
    _A_in = _A_setup()

    def _B_setup():
        B, S, D, F = (1, 2048, 1024, 3584)
        return {'x': _w((lambda *s: _rng.normal(s) * 0.05)(B, S, D)), 'w1': _w((lambda *s: _rng.normal(s) * 0.1)(D, F) * D ** (-0.5)), 'b1': _w((lambda *s: _rng.normal(s) * 0.1)(F) * 0.01), 'w2': _w((lambda *s: _rng.normal(s) * 0.1)(F, D) * F ** (-0.5)), 'b2': _w((lambda *s: _rng.normal(s) * 0.05)(D) * 0.01)}
    _B_in = _B_setup()
    return {'A_x': _A_in['x'], 'A_mem0': _A_in['mem0'], 'A_Wq': _A_in['Wq'], 'A_Wk': _A_in['Wk'], 'A_Wv': _A_in['Wv'], 'A_Wo': _A_in['Wo'], 'A_seg_len': _A_in['seg_len'], 'B_x': _B_in['x'], 'B_w1': _B_in['w1'], 'B_b1': _B_in['b1'], 'B_w2': _B_in['w2'], 'B_b2': _B_in['b2']}

def reference(A_x, A_mem0, A_Wq, A_Wk, A_Wv, A_Wo, A_seg_len, B_x, B_w1, B_b1, B_w2, B_b2):

    def _A_ref(x, mem0, Wq, Wk, Wv, Wo, seg_len):
        B, S, Dm = x.shape
        H, Dh = (Wq.shape[1], Wq.shape[2])
        M = mem0.shape[1]
        scale = Dh ** (-0.5)
        n_seg = S // seg_len
        L = M + seg_len
        idx = jnp.arange(L)
        mask = (idx[:, None] < M) | (idx[:, None] >= idx[None, :])
        mem = mem0
        outs = []
        for s in range(n_seg):
            xs = x[:, s * seg_len:(s + 1) * seg_len, :].copy()
            h = jnp.concatenate([mem, xs], axis=1)
            q = jnp.einsum('btd,dhe->bhte', h, Wq)
            k = jnp.einsum('btd,dhe->bhte', h, Wk)
            v = jnp.einsum('btd,dhe->bhte', h, Wv)
            scores = jnp.einsum('bhqe,bhke->bhqk', q, k) * scale
            scores = jnp.where(mask[None, None], scores, -1000000000.0)
            p = _softmax(scores, axis=-1)
            o = jnp.einsum('bhqk,bhke->bhqe', p, v)
            o = jnp.einsum('bhte,hed->btd', o, Wo)
            mem = o[:, :M, :].copy()
            outs.append(o[:, M:, :])
        return jnp.concatenate(outs, axis=1)

    def _B_ref(x, w1, b1, w2, b2):
        h = jnp.einsum('bsd,df->bsf', x, w1) + b1
        h = _gelu(h)
        return jnp.einsum('bsf,fd->bsd', h, w2) + b2
    x = A_x
    xn = _layernorm(x, axis=-1)
    return x + _A_ref(xn, A_mem0, A_Wq, A_Wk, A_Wv, A_Wo, A_seg_len) + _B_ref(xn, B_w1, B_b1, B_w2, B_b2)
```

```python
import functools
import jax
import jax.numpy as jnp
import numpy as np
from jax import lax
import jax.experimental.pallas as pl
import jax.experimental.pallas.tpu as pltpu

S, DM, H, DH, MEM, SEG, FF = 2048, 1024, 32, 128, 8, 32, 3584
L = MEM + SEG
NSEG = S // SEG
F32 = jnp.float32
BF16 = jnp.bfloat16
U32 = jnp.uint32
NT = (((1,), (1,)), ((), ()))
NN = (((1,), (0,)), ((), ()))
MB = 256
NMB = S // MB
NC = 512
NCH = FF // NC
NPAIR = H // 2
PPI = 3 * NPAIR // NMB
UNROLL = 3
RELAY_SLOT = [0, 1, 2, 3, 3, 4, 5, 6]
LN_SLOT = [0, 2, 4, 5]


def _dot(a, b, dims=NN):
    return lax.dot_general(a, b, dims, preferred_element_type=F32)


def _gelu(x):
    c = np.float32(np.sqrt(2.0 / np.pi))
    return 0.5 * x * (1.0 + jnp.tanh(c * (x + 0.044715 * (x * x * x))))


def _kernel(x_hbm, mem0_hbm, wq_hbm, wk_hbm, wv_hbm, wo_hbm, w1_hbm, b1_hbm, w2_hbm, b2_hbm,
            y_hbm,
            x_vm, xn_vm, h_vm, st_vm, wqkv_vm, wo_vm, w1_vm, w2_vm, o_vm, hcat_vm,
            mem0_vm, b1_vm, b2_vm, b1f_vm, b2f_vm,
            sem_x, sem_w1, sem_p, sem_m, sem_y):
    w_hbm = [wq_hbm.bitcast(U32), wk_hbm.bitcast(U32), wv_hbm.bitcast(U32)]

    def cp_x(i):
        r = pl.ds(i * MB, MB)
        return pltpu.make_async_copy(x_hbm.at[r, :], x_vm.at[r, :], sem_x.at[i])

    def cp_w1(j):
        c = pl.ds(j * NC, NC)
        return pltpu.make_async_copy(w1_hbm.at[:, c], w1_vm.at[:, c], sem_w1.at[j])

    def cp_pair(n):
        m, p = n % 3, n // 3
        return pltpu.make_async_copy(w_hbm[m].at[:, p, 0], st_vm.at[n], sem_p.at[n])

    cp_o = [pltpu.make_async_copy(wo_hbm.bitcast(U32).at[:, pl.ds(j * 128, 128)], wo_vm.at[j], sem_m.at[0]) for j in range(8)]
    cp_2 = [pltpu.make_async_copy(w2_hbm.bitcast(U32).at[:, pl.ds(j * 128, 128)], w2_vm.at[j], sem_m.at[1]) for j in range(8)]
    cp_b1 = pltpu.make_async_copy(b1_hbm, b1_vm, sem_m.at[2])
    cp_b2 = pltpu.make_async_copy(b2_hbm, b2_vm, sem_m.at[3])
    cp_m0 = pltpu.make_async_copy(mem0_hbm, mem0_vm, sem_m.at[4])

    def layernorm(i, t=None):
        r = pl.ds(i * MB, MB) if t is None else pl.ds(i * MB + t * (MB // 4), MB // 4)
        x = x_vm[r, :].astype(F32)
        m = jnp.mean(x, axis=-1, keepdims=True)
        d = x - m
        v = jnp.mean(d * d, axis=-1, keepdims=True)
        xn = d * lax.rsqrt(v + 1e-5)
        xn_vm[r, :] = xn.astype(BF16)

    def relayout(n):
        m, p = n % 3, n // 3
        for g in range(8):
            rows = pl.ds(g * 64, 64)
            a = st_vm[n, pl.ds(g * 128, 64, stride=2), :]
            b = st_vm[n, pl.ds(g * 128 + 1, 64, stride=2), :]
            wqkv_vm[m, 2 * p, rows, :] = (a & jnp.uint32(0xFFFF)) | (b << 16)
            wqkv_vm[m, 2 * p + 1, rows, :] = (a >> 16) | (b & jnp.uint32(0xFFFF0000))

    def ffn1(i, first):
        r = pl.ds(i * MB, MB)
        a = xn_vm[r, :]
        for j in range(NCH):
            if first:
                cp_w1(j).wait()
                if j + 2 < NCH:
                    cp_w1(j + 2).start()
                if j == 1:
                    cp_x(1).wait()
                    cp_x(2).start()
                if j == NCH - 1:
                    cp_x(2).wait()
            cs = pl.ds(j * NC, NC)
            z = _dot(a, w1_vm[:, cs])
            for jj in range(NC // 128):
                n = j * (NC // 128) + jj
                zz = z[:, jj * 128:(jj + 1) * 128] + b1f_vm[n:n + 1, :]
                h_vm[r, n * 128:(n + 1) * 128] = _gelu(zz).astype(BF16)
            if first and j >= 1 and j <= 4:
                layernorm(1, j - 1)

    cp_x(0).start()
    cp_w1(0).start()
    cp_b1.start()
    cp_b2.start()
    cp_m0.start()
    cp_w1(1).start()
    cp_x(0).wait()
    cp_x(1).start()
    layernorm(0)
    cp_b1.wait()
    b1f_vm[...] = b1_vm[...].astype(F32)
    ffn1(0, True)
    for i in range(3, NMB):
        cp_x(i).start()
    ffn1(1, False)
    layernorm(2)
    for i in range(3, NMB):
        cp_x(i).wait()
    for n in range(3 * NPAIR):
        cp_pair(n).start()
    for c in cp_o:
        c.start()
    for c in cp_2:
        c.start()
    for i in range(2, NMB):
        ffn1(i, False)
        if i + 1 < NMB:
            layernorm(i + 1)
    for n in range(3 * NPAIR):
        cp_pair(n).wait()
    for c in cp_o:
        c.wait()
    for c in cp_2:
        c.wait()
    cp_b2.wait()
    cp_m0.wait()
    b2f_vm[...] = b2_vm[...].astype(F32)
    hcat_vm[0:MEM, :] = mem0_vm[...].astype(F32)
    hcat_vm[MEM:L, :] = xn_vm[0:SEG, :].astype(F32)

    row = lax.broadcasted_iota(jnp.int32, (L, L), 0)
    col = lax.broadcasted_iota(jnp.int32, (L, L), 1)
    allowed = (row < MEM) | (row >= col)
    scale = np.float32(DH ** -0.5)

    def step(s, c):
        r = pl.ds(s * SEG, SEG) if isinstance(s, int) else pl.ds(pl.multiple_of(s * SEG, SEG), SEG)
        q = {}; k = {}; v = {}; e = {}; l = {}; f = {}

        def QKV(t):
            hc = hcat_vm[...]
            q[t] = _dot(hc, pltpu.bitcast(wqkv_vm[0, t], BF16))
            k[t] = _dot(hc, pltpu.bitcast(wqkv_vm[1, t], BF16))
            v[t] = _dot(hc, pltpu.bitcast(wqkv_vm[2, t], BF16))

        def SC(h):
            sc = _dot(q[h], k[h], NT) * scale
            sc = jnp.where(allowed, sc, -1e9)
            m = jnp.max(sc, axis=-1, keepdims=True)
            e[h] = jnp.exp(sc - m)
            l[h] = jnp.sum(e[h], axis=-1, keepdims=True)

        def PV(h):
            o = _dot(e[h], v[h]) * pl.reciprocal(l[h], approx=False, full_range=False)
            o_vm[:, h * DH:(h + 1) * DH] = o

        def F(j):
            f[j] = _dot(h_vm[r, :], pltpu.bitcast(w2_vm[j], BF16)) + b2f_vm[j:j + 1, :]

        outs = {}

        def WO(j):
            cs = pl.ds(j * 128, 128)
            out = _dot(o_vm[...], pltpu.bitcast(wo_vm[j], BF16))
            hcat_vm[0:MEM, cs] = out[0:MEM].astype(BF16).astype(F32)
            outs[j] = out[MEM:L]

        def Y(j):
            cs = pl.ds(j * 128, 128)
            y = x_vm[r, cs].astype(F32) + outs[j] + f[j]
            x_vm[r, cs] = y.astype(BF16)

        for t in range(H):
            QKV(t)
            if t >= 1:
                SC(t - 1)
            if t >= 2:
                PV(t - 2)
        nr = pl.ds((s + 1) * SEG, SEG) if isinstance(s, int) else pl.ds(pl.multiple_of(jnp.minimum(s + 1, NSEG - 1) * SEG, SEG), SEG)
        F(0); F(1)
        SC(31); PV(30)
        F(2); F(3)
        PV(31)
        F(4)
        for j in range(8):
            WO(j)
            if j < 5:
                Y(j)
        hcat_vm[MEM:L, :] = xn_vm[nr, :].astype(F32)
        F(5); F(6); F(7)
        Y(5); Y(6); Y(7)
        pltpu.make_async_copy(x_vm.at[r, :], y_hbm.at[r, :], sem_y).start()
        return c

    for n in range(3 * NPAIR):
        relayout(n)
    step(0, 0)
    lax.fori_loop(1, NSEG, step, 0, unroll=UNROLL)
    pltpu.make_async_copy(x_vm, y_hbm, sem_y).wait()


@jax.jit
def pallas_parallel_sum__memory_aug_recurrent_mem_tr__dense_activation_gelu__prompt_kernel(A_x, A_mem0, A_Wq, A_Wk, A_Wv, A_Wo, A_seg_len, B_x, B_w1, B_b1, B_w2, B_b2):
    x = A_x.reshape(S, DM)
    mem0 = A_mem0.reshape(MEM, DM)
    wq = A_Wq.reshape(DM, NPAIR, 2, DH)
    wk = A_Wk.reshape(DM, NPAIR, 2, DH)
    wv = A_Wv.reshape(DM, NPAIR, 2, DH)
    wo = A_Wo.reshape(H * DH, DM)
    any_spec = pl.BlockSpec(memory_space=pl.ANY)
    y = pl.pallas_call(
        _kernel,
        out_shape=jax.ShapeDtypeStruct((S, DM), BF16),
        in_specs=[any_spec] * 10,
        out_specs=any_spec,
        scratch_shapes=[
            pltpu.VMEM((S, DM), BF16),
            pltpu.VMEM((S, DM), BF16),
            pltpu.VMEM((S, FF), BF16),
            pltpu.VMEM((3 * NPAIR, DM, 128), U32),
            pltpu.VMEM((3, H, DM // 2, DH), U32),
            pltpu.VMEM((8, H * DH // 2, 128), U32),
            pltpu.VMEM((DM, FF), BF16),
            pltpu.VMEM((8, FF // 2, 128), U32),
            pltpu.VMEM((L, H * DH), F32),
            pltpu.VMEM((L, DM), F32),
            pltpu.VMEM((MEM, DM), BF16),
            pltpu.VMEM((FF // 128, 128), BF16),
            pltpu.VMEM((DM // 128, 128), BF16),
            pltpu.VMEM((FF // 128, 128), F32),
            pltpu.VMEM((DM // 128, 128), F32),
            pltpu.SemaphoreType.DMA((NMB,)),
            pltpu.SemaphoreType.DMA((NCH,)),
            pltpu.SemaphoreType.DMA((3 * NPAIR,)),
            pltpu.SemaphoreType.DMA((5,)),
            pltpu.SemaphoreType.DMA,
        ],
        compiler_params=pltpu.CompilerParams(vmem_limit_bytes=110 * 2**20),
        name="rmt_ffn",
    )(x, mem0, wq, wk, wv, wo, B_w1, B_b1.reshape(FF // 128, 128), B_w2, B_b2.reshape(DM // 128, 128))
    return y.reshape(1, S, DM)
```

```python
import jax
import jax.numpy as jnp
import numpy as np
from jax import lax
import jax.experimental.pallas as pl
import jax.experimental.pallas.tpu as pltpu

S, DM, H, DH, MEM, SEG, FF = 2048, 1024, 32, 128, 8, 32, 3584
L = MEM + SEG
NSEG = S // SEG
NPAIR = H // 2
MB = 256
NMB = S // MB
NC = 512
NCH = FF // NC
W1_GROUP = (0, 1, 2, 2, 3, 3, 3)

F32 = jnp.float32
BF16 = jnp.bfloat16
U32 = jnp.uint32
NN = (((1,), (0,)), ((), ()))
NT = (((1,), (1,)), ((), ()))


def _dot(a, b, dims=NN):
    return lax.dot_general(a, b, dims, preferred_element_type=F32)


def _gelu(x):
    c = np.float32(np.sqrt(2.0 / np.pi))
    return 0.5 * x * (1.0 + jnp.tanh(c * (x + 0.044715 * (x * x * x))))


def _kernel(x_hbm, mem0_hbm, wq_hbm, wk_hbm, wv_hbm, wo_hbm, w1_hbm, b1_hbm, w2_hbm, b2_hbm,
            y_hbm,
            x_vm, xn_vm, h_vm, st_vm, wqkv_vm, wo_vm, w1_vm, w2_vm, o_vm, hcat_vm,
            mem0_vm, b1_vm, b2_vm, b1f_vm, b2f_vm,
            sem_x, sem_w1, sem_m, sem_y):
    w_u32 = [wq_hbm.bitcast(U32), wk_hbm.bitcast(U32), wv_hbm.bitcast(U32)]
    wo_u32 = wo_hbm.bitcast(U32)
    w2_u32 = w2_hbm.bitcast(U32)

    def cp_x(i):
        r = pl.ds(i * MB, MB)
        sem = sem_w1.at[3] if i == 2 else sem_x.at[min(i, 2)]
        return pltpu.make_async_copy(x_hbm.at[r, :], x_vm.at[r, :], sem)

    def cp_w1(j):
        c = pl.ds(j * NC, NC)
        return pltpu.make_async_copy(w1_hbm.at[:, c], w1_vm.at[:, c], sem_w1.at[W1_GROUP[j]])

    def cp_pair(n):
        m, p = n % 3, n // 3
        return pltpu.make_async_copy(w_u32[m].at[:, p, 0], st_vm.at[n, pl.ds(0, DM)], sem_m.at[0])

    def cp_wo(j):
        return pltpu.make_async_copy(wo_u32.at[:, pl.ds(j * 128, 128)], wo_vm.at[j], sem_m.at[0])

    def cp_w2(j):
        return pltpu.make_async_copy(w2_u32.at[:, pl.ds(j * 128, 128)], w2_vm.at[j], sem_m.at[0])

    def cp_b1():
        return pltpu.make_async_copy(b1_hbm, b1_vm, sem_m.at[1])

    def cp_b2():
        return pltpu.make_async_copy(b2_hbm, b2_vm, sem_m.at[2])

    def cp_mem0():
        return pltpu.make_async_copy(mem0_hbm, mem0_vm, sem_m.at[2])

    def layernorm(i):
        r = pl.ds(i * MB, MB)
        x = x_vm[r, :].astype(F32)
        m = jnp.mean(x, axis=-1, keepdims=True)
        d = x - m
        v = jnp.mean(d * d, axis=-1, keepdims=True)
        xn_vm[r, :] = (d * lax.rsqrt(v + 1e-5)).astype(BF16)

    def ffn1(i, j):
        r = pl.ds(i * MB, MB)
        z = _dot(xn_vm[r, :], w1_vm[:, j * NC:(j + 1) * NC])
        for jj in range(NC // 128):
            n = j * (NC // 128) + jj
            zz = z[:, jj * 128:(jj + 1) * 128] + b1f_vm[n:n + 1, :]
            h_vm[r, n * 128:(n + 1) * 128] = _gelu(zz).astype(BF16)

    def relayout(n):
        m, p = n % 3, n // 3
        for g in range(DM // 128):
            rows = pl.ds(g * 64, 64)
            a = st_vm[n, pl.ds(g * 128, 64, stride=2), :]
            b = st_vm[n, pl.ds(g * 128 + 1, 64, stride=2), :]
            wqkv_vm[m, 2 * p, rows, :] = (a & np.uint32(0xFFFF)) | (b << 16)
            wqkv_vm[m, 2 * p + 1, rows, :] = (a >> 16) | (b & np.uint32(0xFFFF0000))

    cp_x(0).start()
    cp_w1(0).start()
    cp_b1().start()
    cp_b2().start()
    cp_mem0().start()
    cp_x(0).wait()
    cp_x(1).start()
    cp_w1(1).start()
    layernorm(0)
    cp_w1(0).wait()
    cp_b1().wait()
    b1f_vm[...] = b1_vm[...].astype(F32)
    ffn1(0, 0)
    cp_x(1).wait()
    cp_w1(1).wait()
    cp_w1(2).start()
    cp_w1(3).start()
    layernorm(1)
    ffn1(0, 1); ffn1(1, 0); ffn1(1, 1)
    cp_w1(2).wait()
    cp_w1(3).wait()
    for j in (4, 5, 6):
        cp_w1(j).start()
    cp_x(2).start()
    ffn1(0, 2); ffn1(1, 2); ffn1(0, 3); ffn1(1, 3)
    for j in (4, 5, 6):
        cp_w1(j).wait()
    cp_x(2).wait()
    for i in range(3, NMB):
        cp_x(i).start()
    ffn1(0, 4); ffn1(1, 4); ffn1(0, 5)
    for i in range(3, NMB):
        cp_x(i).wait()
    for n in range(3 * NPAIR):
        cp_pair(n).start()
    for j in range(8):
        cp_wo(j).start()
    for j in range(8):
        cp_w2(j).start()
    ffn1(1, 5); ffn1(0, 6); ffn1(1, 6)
    for i in range(2, NMB):
        layernorm(i)
        for j in range(NCH):
            ffn1(i, j)
    for n in range(3 * NPAIR):
        cp_pair(n).wait()
    for j in range(8):
        cp_wo(j).wait()
    for j in range(8):
        cp_w2(j).wait()
    cp_b2().wait()
    cp_mem0().wait()
    b2f_vm[...] = b2_vm[...].astype(F32)
    hcat_vm[0:MEM, :] = mem0_vm[...].astype(F32)
    hcat_vm[MEM:L, :] = xn_vm[0:SEG, :].astype(F32)

    row = lax.broadcasted_iota(jnp.int32, (L, L), 0)
    col = lax.broadcasted_iota(jnp.int32, (L, L), 1)
    allowed_all = (row < MEM) | (row >= col)
    rowx = lax.broadcasted_iota(jnp.int32, (SEG, L), 0) + MEM
    colx = lax.broadcasted_iota(jnp.int32, (SEG, L), 1)
    allowed_x = rowx >= colx
    scale = np.float32(DH ** -0.5)

    def step(s, last=False):
        def rows(t):
            return pl.ds(t * SEG, SEG) if isinstance(t, int) else pl.ds(pl.multiple_of(t * SEG, SEG), SEG)

        r = rows(s)
        q0 = MEM if last else 0
        allowed = allowed_x if last else allowed_all
        q, k, v, e, l, f, outs = {}, {}, {}, {}, {}, {}, {}

        def qkv(h):
            hc = hcat_vm[...]
            q[h] = _dot(hcat_vm[q0:L, :] if last else hc, pltpu.bitcast(wqkv_vm[0, h], BF16))
            k[h] = _dot(hc, pltpu.bitcast(wqkv_vm[1, h], BF16))
            v[h] = _dot(hc, pltpu.bitcast(wqkv_vm[2, h], BF16))

        def scores(h):
            sc = _dot(q[h], k[h], NT) * scale
            sc = jnp.where(allowed, sc, -1e9)
            m = jnp.max(sc, axis=-1, keepdims=True)
            e[h] = jnp.exp(sc - m)
            l[h] = jnp.sum(e[h], axis=-1, keepdims=True)

        def attend(h):
            o = _dot(e[h], v[h]) * pl.reciprocal(l[h], approx=False, full_range=False)
            o_vm[q0:L, h * DH:(h + 1) * DH] = o

        def ffn2(j):
            f[j] = _dot(h_vm[r, :], pltpu.bitcast(w2_vm[j], BF16)) + b2f_vm[j:j + 1, :]

        def out_proj(j):
            out = _dot(o_vm[q0:L, :], pltpu.bitcast(wo_vm[j], BF16))
            if last:
                outs[j] = out
            else:
                hcat_vm[0:MEM, j * 128:(j + 1) * 128] = out[0:MEM].astype(BF16).astype(F32)
                outs[j] = out[MEM:L]

        def finish(j):
            cs = pl.ds(j * 128, 128)
            y = x_vm[r, cs].astype(F32) + outs[j] + f[j]
            x_vm[r, cs] = y.astype(BF16)

        for h in range(H):
            qkv(h)
            if h >= 1:
                scores(h - 1)
            if h >= 2:
                attend(h - 2)
        ffn2(0); ffn2(1)
        scores(H - 1); attend(H - 2)
        ffn2(2); ffn2(3)
        attend(H - 1)
        ffn2(4)
        for j in range(8):
            out_proj(j)
            if j < 5:
                finish(j)
        if not last:
            hcat_vm[MEM:L, :] = xn_vm[rows(s + 1), :].astype(F32)
        for j in range(5, 8):
            ffn2(j)
            finish(j)
        pltpu.make_async_copy(x_vm.at[r, :], y_hbm.at[r, :], sem_y).start()

    def body(s, carry):
        step(s)
        return carry

    for n in range(3 * NPAIR):
        relayout(n)
    step(0)
    lax.fori_loop(1, NSEG - 1, body, 0, unroll=2)
    step(NSEG - 1, last=True)
    pltpu.make_async_copy(x_vm, y_hbm, sem_y).wait()


@jax.jit
def pallas_parallel_sum__memory_aug_recurrent_mem_tr__dense_activation_gelu__prompt_kernel(
    A_x: jax.Array,
    A_mem0: jax.Array,
    A_Wq: jax.Array,
    A_Wk: jax.Array,
    A_Wv: jax.Array,
    A_Wo: jax.Array,
    A_seg_len: int,
    B_x: jax.Array,
    B_w1: jax.Array,
    B_b1: jax.Array,
    B_w2: jax.Array,
    B_b2: jax.Array,
):
    del A_seg_len, B_x
    assert A_x.shape == (1, S, DM) and A_mem0.shape == (1, MEM, DM) and A_Wq.shape == (DM, H, DH)
    assert B_w1.shape == (DM, FF) and B_w2.shape == (FF, DM)
    x = A_x.reshape(S, DM)
    mem0 = A_mem0.reshape(MEM, DM)
    wq = A_Wq.reshape(DM, NPAIR, 2, DH)
    wk = A_Wk.reshape(DM, NPAIR, 2, DH)
    wv = A_Wv.reshape(DM, NPAIR, 2, DH)
    wo = A_Wo.reshape(H * DH, DM)
    b1 = B_b1.reshape(FF // 128, 128)
    b2 = B_b2.reshape(DM // 128, 128)
    any_spec = pl.BlockSpec(memory_space=pl.ANY)
    y = pl.pallas_call(
        _kernel,
        out_shape=jax.ShapeDtypeStruct((S, DM), BF16),
        in_specs=[any_spec] * 10,
        out_specs=any_spec,
        scratch_shapes=[
            pltpu.VMEM((S, DM), BF16),
            pltpu.VMEM((S, DM), BF16),
            pltpu.VMEM((S, FF), BF16),
            pltpu.VMEM((3 * NPAIR, DM + 8, DH), U32),
            pltpu.VMEM((3, H, DM // 2, DH), U32),
            pltpu.VMEM((8, H * DH // 2, 128), U32),
            pltpu.VMEM((DM, FF), BF16),
            pltpu.VMEM((8, FF // 2, 128), U32),
            pltpu.VMEM((L, H * DH), F32),
            pltpu.VMEM((L, DM), F32),
            pltpu.VMEM((MEM, DM), BF16),
            pltpu.VMEM((FF // 128, 128), BF16),
            pltpu.VMEM((DM // 128, 128), BF16),
            pltpu.VMEM((FF // 128, 128), F32),
            pltpu.VMEM((DM // 128, 128), F32),
            pltpu.SemaphoreType.DMA((3,)),
            pltpu.SemaphoreType.DMA((4,)),
            pltpu.SemaphoreType.DMA((3,)),
            pltpu.SemaphoreType.DMA,
        ],
        compiler_params=pltpu.CompilerParams(vmem_limit_bytes=110 * 2**20),
        name="rmt_ffn",
    )(x, mem0, wq, wk, wv, wo, B_w1, b1, B_w2, b2)
    return y.reshape(1, S, DM)
```

```python
import jax
import jax.numpy as jnp
import numpy as np
from jax import lax
import jax.experimental.pallas as pl
import jax.experimental.pallas.tpu as pltpu

S, DM, H, DH, MEM, SEG, FF = 2048, 1024, 32, 128, 8, 32, 3584
L = MEM + SEG
NSEG = S // SEG
NPAIR = H // 2
MB = 256
NMB = S // MB
RB = 48
W1_COLS = (0, 256, 512, 1024, 1536, 2048, 2560, 3072, 3584)
W1_SEM = (1, 3, 4, 5, 5, 6, 6, 7)

F32 = jnp.float32
BF16 = jnp.bfloat16
U32 = jnp.uint32
NN = (((1,), (0,)), ((), ()))
NT = (((1,), (1,)), ((), ()))


def _dot(a, b, dims=NN):
    return lax.dot_general(a, b, dims, preferred_element_type=F32)


def _gelu(x):
    c = np.float32(np.sqrt(2.0 / np.pi))
    return 0.5 * x * (1.0 + jnp.tanh(c * (x + 0.044715 * (x * x * x))))


def _kernel(x_hbm, mem0_hbm, wq_hbm, wk_hbm, wv_hbm, wo_hbm, w1_hbm, b1_hbm, w2_hbm, b2_hbm,
            y_hbm,
            x_vm, xn_vm, h_vm, st_vm, wqkv_vm, wo_vm, w1_vm, w2_vm, o_vm, hcat_vm,
            mem0_vm, b1_vm, b2_vm, b1f_vm, b2f_vm,
            sem_a, sem_m, sem_y):
    w_u32 = [wq_hbm.bitcast(U32), wk_hbm.bitcast(U32), wv_hbm.bitcast(U32)]
    wo_u32 = wo_hbm.bitcast(U32)
    w2_u32 = w2_hbm.bitcast(U32)
    w1_u32 = w1_hbm.bitcast(U32)

    def cp_x(i):
        r = pl.ds(i * MB, MB)
        sem = sem_a.at[0] if i == 0 else sem_a.at[2] if i == 1 else sem_a.at[8]
        return pltpu.make_async_copy(x_hbm.at[r, :], x_vm.at[r, :], sem)

    class _Group:
        def __init__(self, make):
            self.make = make

        def start(self):
            for c in self.make():
                c.start()

        def wait(self):
            for c in self.make():
                c.wait()

    def cp_w1(j):
        return _Group(lambda: [
            pltpu.make_async_copy(w1_u32.at[:, pl.ds(n * 128, 128)], w1_vm.at[n], sem_a.at[W1_SEM[j]])
            for n in range(W1_COLS[j] // 128, W1_COLS[j + 1] // 128)])

    def cp_pair(n):
        m, p = n % 3, n // 3
        return pltpu.make_async_copy(w_u32[m].at[:, p, 0], st_vm.at[n, pl.ds(0, DM)], sem_m.at[0])

    def cp_wo():
        return pltpu.make_async_copy(wo_u32, wo_vm.at[:, pl.ds(0, DM)], sem_m.at[1])

    def cp_w2():
        return pltpu.make_async_copy(w2_u32, w2_vm.at[:, pl.ds(0, DM)], sem_m.at[1])

    def cp_b1():
        return pltpu.make_async_copy(b1_hbm, b1_vm, sem_a.at[1])

    def cp_b2():
        return pltpu.make_async_copy(b2_hbm, b2_vm, sem_a.at[8])

    def cp_mem0():
        return pltpu.make_async_copy(mem0_hbm, mem0_vm, sem_a.at[8])

    def layernorm(r0, nrows):
        r = pl.ds(r0, nrows)
        x = x_vm[r, :].astype(F32)
        m = jnp.mean(x, axis=-1, keepdims=True)
        d = x - m
        v = jnp.mean(d * d, axis=-1, keepdims=True)
        xn_vm[r, :] = (d * lax.rsqrt(v + 1e-5)).astype(BF16)

    def ffn1(r0, nrows, c0, c1):
        r = pl.ds(r0, nrows)
        w = jnp.concatenate([pltpu.bitcast(w1_vm[n], BF16) for n in range(c0 // 128, c1 // 128)], axis=1)
        z = _dot(xn_vm[r, :], w)
        for n in range(c0 // 128, c1 // 128):
            zz = z[:, n * 128 - c0:(n + 1) * 128 - c0] + b1f_vm[n:n + 1, :]
            h_vm[r, n * 128:(n + 1) * 128] = _gelu(zz).astype(BF16)

    def ffn1_chunk(j, blocks=(0, 1)):
        for i in blocks:
            ffn1(i * MB, MB, W1_COLS[j], W1_COLS[j + 1])

    def relayout(n):
        m, p = n % 3, n // 3
        for g in range(DM // 128):
            rows = pl.ds(g * 64, 64)
            a = st_vm[n, pl.ds(g * 128, 64, stride=2), :]
            b = st_vm[n, pl.ds(g * 128 + 1, 64, stride=2), :]
            wqkv_vm[m, 2 * p, rows, :] = (a & np.uint32(0xFFFF)) | (b << 16)
            wqkv_vm[m, 2 * p + 1, rows, :] = (a >> 16) | (b & np.uint32(0xFFFF0000))

    cp_x(0).start()
    cp_w1(0).start()
    cp_b1().start()
    cp_x(1).start()
    for j in range(1, len(W1_COLS) - 1):
        cp_w1(j).start()
    for i in range(2, NMB):
        cp_x(i).start()
    cp_b2().start()
    cp_mem0().start()
    cp_x(0).wait()
    layernorm(0, MB)
    cp_w1(0).wait()
    cp_b1().wait()
    b1f_vm[...] = b1_vm[...].astype(F32)
    ffn1_chunk(0, blocks=(0,))
    cp_x(1).wait()
    layernorm(MB, MB)
    ffn1_chunk(0, blocks=(1,))
    cp_w1(1).wait()
    ffn1_chunk(1)
    cp_w1(2).wait()
    ffn1_chunk(2)
    cp_w1(3).wait()
    cp_w1(4).wait()
    ffn1_chunk(3)
    ffn1_chunk(4)
    cp_w1(5).wait()
    cp_w1(6).wait()
    ffn1_chunk(5)
    ffn1_chunk(6)
    cp_w1(7).wait()
    for i in range(2, NMB):
        cp_x(i).wait()
    cp_b2().wait()
    cp_mem0().wait()
    for n in range(3 * NPAIR):
        cp_pair(n).start()
    cp_wo().start()
    cp_w2().start()
    ffn1_chunk(7)
    for r0 in range(2 * MB, S, RB):
        layernorm(r0, RB)
        ffn1(r0, RB, 0, FF)
    for n in range(3 * NPAIR):
        cp_pair(n).wait()
    cp_wo().wait()
    cp_w2().wait()
    b2f_vm[...] = b2_vm[...].astype(F32)
    hcat_vm[0:MEM, :] = mem0_vm[...].astype(F32)
    hcat_vm[MEM:L, :] = xn_vm[0:SEG, :].astype(F32)

    row = lax.broadcasted_iota(jnp.int32, (L, L), 0)
    col = lax.broadcasted_iota(jnp.int32, (L, L), 1)
    allowed_all = (row < MEM) | (row >= col)
    rowx = lax.broadcasted_iota(jnp.int32, (SEG, L), 0) + MEM
    colx = lax.broadcasted_iota(jnp.int32, (SEG, L), 1)
    allowed_x = rowx >= colx
    scale = np.float32(DH ** -0.5)

    def step(s, last=False):
        def rows(t):
            return pl.ds(t * SEG, SEG) if isinstance(t, int) else pl.ds(pl.multiple_of(t * SEG, SEG), SEG)

        r = rows(s)
        q0 = MEM if last else 0
        allowed = allowed_x if last else allowed_all
        q, k, v, e, l, f, outs = {}, {}, {}, {}, {}, {}, {}

        def qkv(h):
            hc = hcat_vm[...]
            q[h] = _dot(hcat_vm[q0:L, :] if last else hc, pltpu.bitcast(wqkv_vm[0, h], BF16))
            k[h] = _dot(hc, pltpu.bitcast(wqkv_vm[1, h], BF16))
            v[h] = _dot(hc, pltpu.bitcast(wqkv_vm[2, h], BF16))

        def scores(h):
            sc = _dot(q[h], k[h], NT) * scale
            sc = jnp.where(allowed, sc, -1e9)
            m = jnp.max(sc, axis=-1, keepdims=True)
            e[h] = jnp.exp(sc - m)
            l[h] = jnp.sum(e[h], axis=-1, keepdims=True)

        def attend(h):
            o = _dot(e[h], v[h]) * pl.reciprocal(l[h], approx=False, full_range=False)
            o_vm[q0:L, h * DH:(h + 1) * DH] = o

        def ffn2(j):
            f[j] = _dot(h_vm[r, :], pltpu.bitcast(w2_vm[:, j * 128:(j + 1) * 128], BF16)) + b2f_vm[j:j + 1, :]

        def out_proj(j):
            out = _dot(o_vm[q0:L, :], pltpu.bitcast(wo_vm[:, j * 128:(j + 1) * 128], BF16))
            if last:
                outs[j] = out
            else:
                hcat_vm[0:MEM, j * 128:(j + 1) * 128] = out[0:MEM].astype(BF16).astype(F32)
                outs[j] = out[MEM:L]

        def finish(j):
            cs = pl.ds(j * 128, 128)
            y = x_vm[r, cs].astype(F32) + outs[j] + f[j]
            x_vm[r, cs] = y.astype(BF16)

        for h in range(H):
            qkv(h)
            if h >= 1:
                scores(h - 1)
            if h >= 2:
                attend(h - 2)
        ffn2(0); ffn2(1)
        scores(H - 1); attend(H - 2)
        ffn2(2); ffn2(3)
        attend(H - 1)
        ffn2(4)
        for j in range(8):
            out_proj(j)
            if j < 5:
                finish(j)
        if not last:
            hcat_vm[MEM:L, :] = xn_vm[rows(s + 1), :].astype(F32)
        for j in range(5, 8):
            ffn2(j)
            finish(j)
        pltpu.make_async_copy(x_vm.at[r, :], y_hbm.at[r, :], sem_y).start()

    def body(s, carry):
        step(s)
        return carry

    for n in range(3 * NPAIR):
        relayout(n)
    step(0)
    step(1)
    lax.fori_loop(2, NSEG - 2, body, 0, unroll=3)
    step(NSEG - 2)
    step(NSEG - 1, last=True)
    pltpu.make_async_copy(x_vm, y_hbm, sem_y).wait()


@jax.jit
def pallas_parallel_sum__memory_aug_recurrent_mem_tr__dense_activation_gelu__prompt_kernel(
    A_x: jax.Array,
    A_mem0: jax.Array,
    A_Wq: jax.Array,
    A_Wk: jax.Array,
    A_Wv: jax.Array,
    A_Wo: jax.Array,
    A_seg_len: int,
    B_x: jax.Array,
    B_w1: jax.Array,
    B_b1: jax.Array,
    B_w2: jax.Array,
    B_b2: jax.Array,
):
    del A_seg_len, B_x
    assert A_x.shape == (1, S, DM) and A_mem0.shape == (1, MEM, DM) and A_Wq.shape == (DM, H, DH)
    assert B_w1.shape == (DM, FF) and B_w2.shape == (FF, DM)
    x = A_x.reshape(S, DM)
    mem0 = A_mem0.reshape(MEM, DM)
    wq = A_Wq.reshape(DM, NPAIR, 2, DH)
    wk = A_Wk.reshape(DM, NPAIR, 2, DH)
    wv = A_Wv.reshape(DM, NPAIR, 2, DH)
    wo = A_Wo.reshape(H * DH, DM)
    b1 = B_b1.reshape(FF // 128, 128)
    b2 = B_b2.reshape(DM // 128, 128)
    any_spec = pl.BlockSpec(memory_space=pl.ANY)
    y = pl.pallas_call(
        _kernel,
        out_shape=jax.ShapeDtypeStruct((S, DM), BF16),
        in_specs=[any_spec] * 10,
        out_specs=any_spec,
        scratch_shapes=[
            pltpu.VMEM((S, DM), BF16),
            pltpu.VMEM((S, DM), BF16),
            pltpu.VMEM((S, FF), BF16),
            pltpu.VMEM((3 * NPAIR, DM + 8, DH), U32),
            pltpu.VMEM((3, H, DM // 2, DH), U32),
            pltpu.VMEM((H * DH // 2, DM + 128), U32),
            pltpu.VMEM((FF // 128, DM // 2, 128), U32),
            pltpu.VMEM((FF // 2, DM + 128), U32),
            pltpu.VMEM((L, H * DH), F32),
            pltpu.VMEM((L, DM), F32),
            pltpu.VMEM((MEM, DM), BF16),
            pltpu.VMEM((FF // 128, 128), BF16),
            pltpu.VMEM((DM // 128, 128), BF16),
            pltpu.VMEM((FF // 128, 128), F32),
            pltpu.VMEM((DM // 128, 128), F32),
            pltpu.SemaphoreType.DMA((9,)),
            pltpu.SemaphoreType.DMA((2,)),
            pltpu.SemaphoreType.DMA,
        ],
        compiler_params=pltpu.CompilerParams(vmem_limit_bytes=110 * 2**20),
        name="rmt_ffn",
    )(x, mem0, wq, wk, wv, wo, B_w1, b1, B_w2, b2)
    return y.reshape(1, S, DM)
```
